```python
import os as _os
_os.environ.setdefault("JAX_PLATFORMS", "cpu")
import jax
import jax.numpy as jnp

def _softmax(x, axis=-1):
    return jax.nn.softmax(x, axis=axis)
def _gelu(x):
    return jax.nn.gelu(x, approximate=True)
def _silu(x):
    return jax.nn.silu(x)
def _sigmoid(x):
    return jax.nn.sigmoid(x)
def _layernorm(x, axis=-1, eps=1e-5):
    m = jnp.mean(x, axis=axis, keepdims=True)
    v = jnp.var(x, axis=axis, keepdims=True)
    return (x - m) / jnp.sqrt(v + eps)
def _scatter_add(tgt, idx, src, axis=0):
    return tgt.at[idx].add(src)
def _segment_sum(src, seg, n):
    return jax.ops.segment_sum(src, seg, n)
class _Rng:
    def __init__(self, key):
        self._k = key
    def _next(self):
        self._k, sub = jax.random.split(self._k)
        return sub
    def normal(self, shape):
        return jax.random.normal(self._next(), shape, dtype=jnp.bfloat16)
    def randint(self, lo, hi, shape):
        return jax.random.randint(self._next(), shape, lo, hi, dtype=jnp.int32)
    def uniform(self, shape, lo=0.0, hi=1.0):
        return jax.random.uniform(self._next(), shape, jnp.bfloat16, lo, hi)
    def permutation(self, n):
        return jax.random.permutation(self._next(), n)


kernel_name = 'sequential_preLN__sliding_block__dense_activation_gelu__prompt'

def setup_inputs():
    _rng = _Rng(jax.random.key(int.from_bytes(__import__("os").urandom(4), "little")))
    _w = (lambda a: (lambda t: t.astype(jnp.bfloat16) if jnp.issubdtype(t.dtype, jnp.floating) else t)(jnp.asarray(a)))
    def _A_setup():
        B, S, D = 1, 2048, 640
        return {
            "x": _w((lambda *s: _rng.normal(s) * 0.05)(B, S, D)),
            "wqkv": _w((lambda *s: _rng.normal(s) * 0.05)(D, 3 * D)),
            "wo": _w((lambda *s: _rng.normal(s) * 0.05)(D, D)),
        }
    _A_in = _A_setup()

    def _B_setup():
        B, S, D, F = 1, 2048, 640, 1536
        return {
            "x": _w((lambda *s: _rng.normal(s) * 0.05)(B, S, D)),
            "w1": _w((lambda *s: _rng.normal(s) * 0.8)(D, F) * (D ** -0.5)),
            "b1": _w((lambda *s: _rng.normal(s) * 0.8)(F) * 0.01),
            "w2": _w((lambda *s: _rng.normal(s) * 0.8)(F, D) * (F ** -0.5)),
            "b2": _w((lambda *s: _rng.normal(s) * 0.05)(D) * 0.01),
        }
    _B_in = _B_setup()

    return {
        "A_x": _A_in["x"],
        "A_wqkv": _A_in["wqkv"],
        "A_wo": _A_in["wo"],
        "B_x": _B_in["x"],
        "B_w1": _B_in["w1"],
        "B_b1": _B_in["b1"],
        "B_w2": _B_in["w2"],
        "B_b2": _B_in["b2"],
    }

def reference(A_x, A_wqkv, A_wo, B_x, B_w1, B_b1, B_w2, B_b2):
    def _A_ref(x, wqkv, wo):
        B, S, D = x.shape
        H = 32; Dh = D // H; W = 256
        qkv = (lambda x, *d: x.transpose(*d))((x @ wqkv).reshape(B, S, 3, H, Dh), 2, 0, 3, 1, 4)
        q, k, v = qkv[0], qkv[1], qkv[2]
        scores = jnp.einsum("bhqd,bhkd->bhqk", q, k) * (Dh ** -0.5)
        idx = jnp.arange(S)
        mask = (idx[:, None] - idx[None, :] >= 0) & (idx[:, None] - idx[None, :] < W)
        scores = jnp.where(mask[None, None], scores, -1e9)
        p = _softmax(scores, axis=-1)
        o = jnp.einsum("bhqk,bhkd->bhqd", p, v)
        return (lambda x, *d: x.transpose(*d))(o, 0, 2, 1, 3).reshape(B, S, D) @ wo

    def _B_ref(x, w1, b1, w2, b2):
        h = jnp.einsum("bsd,df->bsf", x, w1) + b1
        h = _gelu(h)
        return jnp.einsum("bsf,fd->bsd", h, w2) + b2

    x = A_x
    h = x + _A_ref(_layernorm(x, axis=-1), A_wqkv, A_wo)
    h2 = h + _B_ref(_layernorm(h, axis=-1), B_w1, B_b1, B_w2, B_b2)
    return h2
```

```python
import functools
import math

import jax
import jax.numpy as jnp
import jax.experimental.pallas as pl
import jax.experimental.pallas.tpu as pltpu

H = 32
TQ = 128
TB = 256
G = 4
AHEAD = 3
NCH = 3
LN_EPS = 1e-5
NEG = -1e30
LOG2E = 1.4426950408889634
BF16 = jnp.bfloat16
F32 = jnp.float32
I32 = jnp.int32

FIRST = '+0,wk x +wq l -wk +wv k -wq +1,wo p q -wv +w1,w2,b1,b2 v'
SECOND = 'a0 x -wo l o k h p q v -w1,w2,b1,b2 X'
BODY = 'x l f f f f a f q v o k p h f s'
LAST = 'f f f a f o f h f s'


def _iota(rows, dim):
    return jax.lax.broadcasted_iota(I32, (rows, 128), dim)


def _bits(x):
    return pltpu.bitcast(x, I32)


def _unbits(x):
    return pltpu.bitcast(x, BF16)


def _dot(a, b):
    return jax.lax.dot_general(a, b, (((1,), (0,)), ((), ())), preferred_element_type=F32)


def _layernorm(x):
    m = jnp.mean(x, axis=-1, keepdims=True)
    xc = x - m
    v = jnp.mean(xc * xc, axis=-1, keepdims=True)
    return xc * jax.lax.rsqrt(v + LN_EPS)


def _gelu(x):
    c = math.sqrt(2.0 / math.pi)
    u = x * (c + (c * 0.044715) * (x * x))
    hx = 0.5 * x
    return hx + hx * jnp.tanh(u)


def _kernel(x_hbm, wqkv_hbm, wo_hbm, w1_hbm, b1_hbm, w2_hbm, b2_hbm, o_hbm,
            x_ref, wk_ref, wq_ref, wv_ref, wo_ref, w1_ref, w2_ref, b1_ref, b2_ref,
            kb_ref, krep_ref, qb_ref, vt_ref, ot_ref, att_ref, h_ref, hn_ref, o_ref,
            wsem, xsem, osem, *, T, D, DH, NS):
    NT = T // TQ
    weights = dict(
        wk=(wqkv_hbm.at[:, D:2 * D], wk_ref),
        wq=(wqkv_hbm.at[:, 0:D], wq_ref),
        wv=(wqkv_hbm.at[:, 2 * D:3 * D], wv_ref),
        wo=(wo_hbm, wo_ref),
        w1=(w1_hbm, w1_ref),
        w2=(w2_hbm, w2_ref),
        b1=(b1_hbm, b1_ref),
        b2=(b2_hbm, b2_ref),
    )

    def rows_of(blk):
        return pl.ds(blk * T if isinstance(blk, int) else pl.multiple_of(blk * T, T), T)

    def x_dma(blk):
        return pltpu.make_async_copy(x_hbm.at[rows_of(blk)], x_ref.at[rows_of(blk)], xsem.at[blk])

    def out_dma(blk):
        return pltpu.make_async_copy(o_ref.at[rows_of(blk)], o_hbm.at[rows_of(blk)], osem.at[blk])

    def dma(name):
        if name.isdigit():
            return x_dma(int(name))
        return pltpu.make_async_copy(*weights[name], wsem.at[list(weights).index(name)])

    def tile(ref, blk, t):
        return ref.at[(blk if t >= 0 else blk + 1) & 1, t % NT]

    def ln1(blk):
        return _layernorm(x_ref[rows_of(blk), :].astype(F32)).astype(BF16)

    def replicate_keys(blk, t):
        lane = _iota(64, 1)
        rows = slice(t * 64, (t + 1) * 64)
        for h0 in range(0, H, 3):
            nh = min(3, H - h0)
            w0 = DH * h0
            ja, jb = w0 // 128, (w0 + nh * DH - 1) // 128
            xw = kb_ref[rows, ja * 128:(ja + 1) * 128]
            if ja != jb:
                xw = jnp.where(lane >= w0 - ja * 128, xw, kb_ref[rows, jb * 128:(jb + 1) * 128])
            y = jnp.where(((lane - w0) & 64) == 0, xw, pltpu.roll(xw, 64, 1))
            y32 = pltpu.roll(y, 32, 1)
            for h in range(h0, h0 + nh):
                tile(krep_ref, blk, t)[h] = jnp.where(((lane - DH * h) & 32) == 0, y, y32)

    def qk(blk, t, h, ntiles):
        seg = _iota(16, 1) >> 5
        k_last = tile(krep_ref, blk, t)[h]
        if ntiles == 3:
            k_first = tile(krep_ref, blk, t - 2)[h]
            diag = k_last[0:16]
            for s in (1, 2, 3):
                diag = jnp.where(seg == s, k_last[16 * s:16 * s + 16], diag)
            ring = jnp.where((_iota(48, 1) >> 5) <= (_iota(48, 0) >> 4),
                             k_first[0:48], k_last[0:48])
            lhs = [diag, ring, k_first[48:64]]
        else:
            lhs = [k_last]
        if ntiles > 1:
            lhs.append(tile(krep_ref, blk, t - 1)[h])
        cols = slice(t * TQ, (t + 1) * TQ)
        a = DH * h // 32 * 32
        o = DH * h - a
        row = _iota(16, 0)
        w = qb_ref[a // 2:a // 2 + 16, cols]
        if o + DH > 32:
            w = jnp.where(row >= o // 2, w, qb_ref[a // 2 + 16:a // 2 + 32, cols])
        w = jnp.where(((row - o // 2) & 15) < DH // 2, w, 0)
        wb = jnp.concatenate([jnp.where(seg == s, w, 0) for s in range(4)], axis=0)
        return _dot(_unbits(jnp.concatenate(lhs, axis=0)), _unbits(wb))

    def softmax_numerators(sc, ntiles):
        r, q = _iota(128, 0), _iota(128, 1)
        if ntiles == 3:
            use_diag = ((r >> 5) == (q >> 5)) & (r <= q)
            s_ring = jnp.where(use_diag, jnp.concatenate([sc[0:32]] * 4, axis=0), sc[32:160])
            s_mid = sc[160:288]
        else:
            s_ring = jnp.where(r <= q, sc[0:128], NEG)
            s_mid = sc[128:256] if ntiles == 2 else None
        m = s_ring if s_mid is None else jnp.maximum(s_ring, s_mid)
        m = jnp.max(m, axis=0, keepdims=True)
        ps = [] if s_mid is None else [jnp.exp2(s_mid - m)]
        p_ring = jnp.exp2(s_ring - m)
        if ntiles == 3:
            first = r > q
            ps += [jnp.where(first, p_ring, 0.0), jnp.where(first, 0.0, p_ring)]
        else:
            ps += [p_ring]
        return jnp.concatenate(ps, axis=0).astype(BF16)

    def pv(blk, t, h, p, ntiles):
        va = DH * h // 8 * 8
        low = _iota(8, 0) < 4
        vs = []
        for tt in [t - 1, t - 2][:ntiles - 1] + [t]:
            vt = tile(vt_ref, blk, tt)
            if h % 2 == 0:
                vs.append(jnp.concatenate(
                    [vt[va:va + 16, :], jnp.where(low, vt[va + 16:va + 24, :], 1.0)], axis=0))
            else:
                vs.append(jnp.concatenate(
                    [jnp.where(low, 1.0, vt[va:va + 8, :]), vt[va + 8:va + 24, :]], axis=0))
        ov = _dot(jnp.concatenate(vs, axis=1), p)
        lrow = 23 if h % 2 == 0 else 0
        rinv = 1.0 / jnp.broadcast_to(ov[lrow:lrow + 1], (8, 128))
        return ov * jnp.concatenate([rinv] * 3, axis=0)

    def attention(blk, ntiles):
        groups = [(t, h0) for t in range(NT) for h0 in range(0, H, G)]

        def qk_group(t, h0):
            return [qk(blk, t, h0 + i, ntiles[t]) for i in range(G)]

        scs = [qk_group(*groups[i]) for i in range(AHEAD)]
        done = 0
        for gi, (t, h0) in enumerate(groups):
            ps = [softmax_numerators(sc, ntiles[t]) for sc in scs[gi]]
            if gi + AHEAD < len(groups):
                scs.append(qk_group(*groups[gi + AHEAD]))
            outs = [pv(blk, t, h0 + i, ps[i], ntiles[t]) for i in range(G)]
            for i in range(0, G, 2):
                e, f = outs[i], outs[i + 1]
                shared = jnp.where(_iota(8, 0) < 4, e[16:24], f[0:8])
                ot_ref[t, DH * (h0 + i):DH * (h0 + i + 2), :] = jnp.concatenate(
                    [e[0:16], shared, f[8:24]], axis=0)
            done = 0 if h0 == 0 else done
            while (done + 1) * 128 <= DH * (h0 + G):
                cs = slice(done * 128, (done + 1) * 128)
                att_ref[t * TQ:(t + 1) * TQ, cs] = ot_ref[t, cs, :].T.astype(BF16)
                done += 1

    def mlp_stages(blk):
        fc = w1_ref.shape[1] // NCH
        b1 = b1_ref[...].astype(F32)[None, :]
        gs, acc = [], []

        def up(c):
            cs = slice(c * fc, (c + 1) * fc)
            gs.append(_gelu(_dot(hn_ref[...], w1_ref[:, cs]) + b1[:, cs]).astype(BF16))

        def down(c):
            if c == 0:
                acc.append(h_ref[...] + b2_ref[...].astype(F32)[None, :])
            acc[0] = acc[0] + _dot(gs[c], w2_ref[c * fc:(c + 1) * fc, :])
            if c == NCH - 1:
                o_ref[rows_of(blk), :] = acc[0].astype(o_ref.dtype)

        return ([functools.partial(up, c) for c in range(NCH)]
                + [functools.partial(down, c) for c in range(NCH)])

    def run(prog, i):
        prog = prog.split()
        stages = mlp_stages(i - 1) if "f" in prog else []
        xn = hres = None
        for op in prog:
            if op[0] == "+":
                for name in op[1:].split(","):
                    dma(name).start()
            elif op[0] == "-":
                for name in op[1:].split(","):
                    dma(name).wait()
            elif op == "x":
                x_dma(i + 1).wait()
            elif op == "X":
                for blk in range(2, NS):
                    x_dma(blk).start()
            elif op == "l":
                xn = ln1(i + 1)
            elif op == "k":
                kb_ref[...] = _bits(_dot(xn, wk_ref[...]).astype(BF16))
            elif op == "p":
                for t in range(NT):
                    replicate_keys(i + 1, t)
            elif op == "q":
                q = _dot(xn, wq_ref[...]) * (DH ** -0.5 * LOG2E)
                qb_ref[...] = _bits(q.T.astype(BF16))
            elif op == "v":
                v = _dot(xn, wv_ref[...])
                for t in range(NT):
                    tile(vt_ref, i + 1, t)[...] = v[t * TQ:(t + 1) * TQ].T
            elif op == "a":
                attention(i, [3] * NT)
            elif op == "a0":
                attention(i, [min(t + 1, 3) for t in range(NT)])
            elif op == "o":
                hres = x_ref[rows_of(i), :].astype(F32) + _dot(att_ref[...], wo_ref[...])
            elif op == "h":
                h_ref[...] = hres
                hn_ref[...] = _layernorm(hres).astype(BF16)
            elif op == "f":
                stages.pop(0)()
            elif op == "s":
                out_dma(i - 1).start()

    def body(i, carry):
        run(BODY, i)
        return carry

    run(FIRST, -1)
    run(SECOND, 0)
    jax.lax.fori_loop(1, NS - 1, body, 0)
    run(LAST, NS - 1)
    run("f " * (2 * NCH) + "s", NS)
    for blk in range(NS):
        out_dma(blk).wait()


@jax.jit
def pallas_sequential_preLN__sliding_block__dense_activation_gelu__prompt_kernel(
    A_x: jax.Array,
    A_wqkv: jax.Array,
    A_wo: jax.Array,
    B_x: jax.Array,
    B_w1: jax.Array,
    B_b1: jax.Array,
    B_w2: jax.Array,
    B_b2: jax.Array,
):
    del B_x
    B, S, D = A_x.shape
    F = B_w1.shape[1]
    T = TB
    NS, NT = S // T, T // TQ
    hbm = pl.BlockSpec(memory_space=pl.ANY)
    out = pl.pallas_call(
        functools.partial(_kernel, T=T, D=D, DH=D // H, NS=NS),
        in_specs=[hbm] * 7,
        out_specs=hbm,
        out_shape=jax.ShapeDtypeStruct((S, D), A_x.dtype),
        scratch_shapes=[
            pltpu.VMEM((S, D), BF16),
            pltpu.VMEM((D, D), BF16),
            pltpu.VMEM((D, D), BF16),
            pltpu.VMEM((D, D), BF16),
            pltpu.VMEM((D, D), BF16),
            pltpu.VMEM((D, F), BF16),
            pltpu.VMEM((F, D), BF16),
            pltpu.VMEM((F,), BF16),
            pltpu.VMEM((D,), BF16),
            pltpu.VMEM((T // 2, D), I32),
            pltpu.VMEM((2, NT, H, TQ // 2, 128), I32),
            pltpu.VMEM((D // 2, T), I32),
            pltpu.VMEM((2, NT, D, TQ), F32),
            pltpu.VMEM((NT, D, TQ), F32),
            pltpu.VMEM((T, D), BF16),
            pltpu.VMEM((T, D), F32),
            pltpu.VMEM((T, D), BF16),
            pltpu.VMEM((S, D), A_x.dtype),
            pltpu.SemaphoreType.DMA((8,)),
            pltpu.SemaphoreType.DMA((NS,)),
            pltpu.SemaphoreType.DMA((NS,)),
        ],
        compiler_params=pltpu.CompilerParams(
            flags={"XLA_TPU_EVENLY_DISTRIBUTE_CRITICAL_NODES": True},
            vmem_limit_bytes=64 * 1024 * 1024,
        ),
    )(A_x.reshape(S, D), A_wqkv, A_wo, B_w1, B_b1, B_w2, B_b2)
    return out.reshape(B, S, D)
```

```python
import functools
import math

import jax
import jax.numpy as jnp
import jax.experimental.pallas as pl
import jax.experimental.pallas.tpu as pltpu

H = 32
TQ = 128
TB = 256
G = 4
AHEAD = 3
NCH = 3
LN_EPS = 1e-5
NEG = -1e30
LOG2E = 1.4426950408889634
BF16 = jnp.bfloat16
F32 = jnp.float32
I32 = jnp.int32

FIRST = '+0,wk x +wq l -wk +wv k -wq +1,wo p q -wv +w1,w2,b1,b2,2 v'
SECOND = 'a0 x -wo l o k h p q v -w1,w2,b1,b2 X'
BODY = 'x l f f f 13@f a f q v o k p h f s'
LAST = 'f f f 13@f a f o h f s'


def _iota(rows, dim):
    return jax.lax.broadcasted_iota(I32, (rows, 128), dim)


def _bits(x):
    return pltpu.bitcast(x, I32)


def _unbits(x):
    return pltpu.bitcast(x, BF16)


def _dot(a, b):
    return jax.lax.dot_general(a, b, (((1,), (0,)), ((), ())), preferred_element_type=F32)


def _layernorm(x):
    m = jnp.mean(x, axis=-1, keepdims=True)
    xc = x - m
    v = jnp.mean(xc * xc, axis=-1, keepdims=True)
    return xc * jax.lax.rsqrt(v + LN_EPS)


def _gelu(x):
    c = math.sqrt(2.0 / math.pi)
    u = x * (c + (c * 0.044715) * (x * x))
    hx = 0.5 * x
    return hx + hx * jnp.tanh(u)


def _kernel(x_hbm, wqkv_hbm, wo_hbm, w1_hbm, b1_hbm, w2_hbm, b2_hbm, o_hbm,
            x_ref, wk_ref, wq_ref, wv_ref, wo_ref, w1_ref, w2_ref, b1_ref, b2_ref,
            kb_ref, krep_ref, qb_ref, vt_ref, ot_ref, att_ref, h_ref, hn_ref, o_ref,
            wsem, xsem, osem, *, T, D, DH, NS):
    NT = T // TQ
    weights = dict(
        wk=(wqkv_hbm.at[:, D:2 * D], wk_ref),
        wq=(wqkv_hbm.at[:, 0:D], wq_ref),
        wv=(wqkv_hbm.at[:, 2 * D:3 * D], wv_ref),
        wo=(wo_hbm, wo_ref),
        w1=(w1_hbm, w1_ref),
        w2=(w2_hbm, w2_ref),
        b1=(b1_hbm, b1_ref),
        b2=(b2_hbm, b2_ref),
    )

    def rows_of(blk):
        return pl.ds(blk * T if isinstance(blk, int) else pl.multiple_of(blk * T, T), T)

    def x_dma(blk):
        return pltpu.make_async_copy(x_hbm.at[rows_of(blk)], x_ref.at[rows_of(blk)], xsem.at[blk])

    def out_dma(blk):
        return pltpu.make_async_copy(o_ref.at[rows_of(blk)], o_hbm.at[rows_of(blk)], osem.at[blk])

    def dma(name):
        if name.isdigit():
            return x_dma(int(name))
        return pltpu.make_async_copy(*weights[name], wsem.at[list(weights).index(name)])

    def tile(ref, blk, t):
        return ref.at[(blk if t >= 0 else blk + 1) & 1, t % NT]

    def ln1(blk):
        return _layernorm(x_ref[rows_of(blk), :].astype(F32)).astype(BF16)

    def replicate_keys(blk, t):
        lane = _iota(64, 1)
        rows = slice(t * 64, (t + 1) * 64)
        for h0 in range(0, H, 3):
            nh = min(3, H - h0)
            w0 = DH * h0
            ja, jb = w0 // 128, (w0 + nh * DH - 1) // 128
            xw = kb_ref[rows, ja * 128:(ja + 1) * 128]
            if ja != jb:
                xw = jnp.where(lane >= w0 - ja * 128, xw, kb_ref[rows, jb * 128:(jb + 1) * 128])
            y = jnp.where(((lane - w0) & 64) == 0, xw, pltpu.roll(xw, 64, 1))
            y32 = pltpu.roll(y, 32, 1)
            for h in range(h0, h0 + nh):
                tile(krep_ref, blk, t)[h] = jnp.where(((lane - DH * h) & 32) == 0, y, y32)

    def qk(blk, t, h, ntiles):
        seg = _iota(16, 1) >> 5
        k_last = tile(krep_ref, blk, t)[h]
        if ntiles == 3:
            k_first = tile(krep_ref, blk, t - 2)[h]
            diag = k_last[0:16]
            for s in (1, 2, 3):
                diag = jnp.where(seg == s, k_last[16 * s:16 * s + 16], diag)
            ring = jnp.where((_iota(48, 1) >> 5) <= (_iota(48, 0) >> 4),
                             k_first[0:48], k_last[0:48])
            lhs = [diag, ring, k_first[48:64]]
        else:
            lhs = [k_last]
        if ntiles > 1:
            lhs.append(tile(krep_ref, blk, t - 1)[h])
        cols = slice(t * TQ, (t + 1) * TQ)
        a = DH * h // 32 * 32
        o = DH * h - a
        row = _iota(16, 0)
        w = qb_ref[a // 2:a // 2 + 16, cols]
        if o + DH > 32:
            w = jnp.where(row >= o // 2, w, qb_ref[a // 2 + 16:a // 2 + 32, cols])
        w = jnp.where(((row - o // 2) & 15) < DH // 2, w, 0)
        wb = jnp.concatenate([jnp.where(seg == s, w, 0) for s in range(4)], axis=0)
        return _dot(_unbits(jnp.concatenate(lhs, axis=0)), _unbits(wb))

    def softmax_numerators(sc, ntiles):
        r, q = _iota(128, 0), _iota(128, 1)
        if ntiles == 3:
            use_diag = ((r >> 5) == (q >> 5)) & (r <= q)
            s_ring = jnp.where(use_diag, jnp.concatenate([sc[0:32]] * 4, axis=0), sc[32:160])
            s_mid = sc[160:288]
        else:
            s_ring = jnp.where(r <= q, sc[0:128], NEG)
            s_mid = sc[128:256] if ntiles == 2 else None
        m = s_ring if s_mid is None else jnp.maximum(s_ring, s_mid)
        m = jnp.max(m, axis=0, keepdims=True)
        ps = [] if s_mid is None else [jnp.exp2(s_mid - m)]
        p_ring = jnp.exp2(s_ring - m)
        if ntiles == 3:
            first = r > q
            ps += [jnp.where(first, p_ring, 0.0), jnp.where(first, 0.0, p_ring)]
        else:
            ps += [p_ring]
        return jnp.concatenate(ps, axis=0).astype(BF16)

    def pv(blk, t, h, p, ntiles):
        va = DH * h // 8 * 8
        low = _iota(8, 0) < 4
        vs = []
        for tt in [t - 1, t - 2][:ntiles - 1] + [t]:
            vt = tile(vt_ref, blk, tt)
            if h % 2 == 0:
                vs.append(jnp.concatenate(
                    [vt[va:va + 16, :], jnp.where(low, vt[va + 16:va + 24, :], 1.0)], axis=0))
            else:
                vs.append(jnp.concatenate(
                    [jnp.where(low, 1.0, vt[va:va + 8, :]), vt[va + 8:va + 24, :]], axis=0))
        ov = _dot(jnp.concatenate(vs, axis=1), p)
        lrow = 23 if h % 2 == 0 else 0
        rinv = 1.0 / jnp.broadcast_to(ov[lrow:lrow + 1], (8, 128))
        return ov * jnp.concatenate([rinv] * 3, axis=0)

    def attention(blk, ntiles, fill):
        groups = [(t, h0) for t in range(NT) for h0 in range(0, H, G)]

        def qk_group(t, h0):
            return [qk(blk, t, h0 + i, ntiles[t]) for i in range(G)]

        scs = [qk_group(*groups[i]) for i in range(AHEAD)]
        done = 0
        for gi, (t, h0) in enumerate(groups):
            ps = [softmax_numerators(sc, ntiles[t]) for sc in scs[gi]]
            if gi + AHEAD < len(groups):
                scs.append(qk_group(*groups[gi + AHEAD]))
            if gi in fill:
                fill[gi]()
            outs = [pv(blk, t, h0 + i, ps[i], ntiles[t]) for i in range(G)]
            for i in range(0, G, 2):
                e, f = outs[i], outs[i + 1]
                shared = jnp.where(_iota(8, 0) < 4, e[16:24], f[0:8])
                ot_ref[t, DH * (h0 + i):DH * (h0 + i + 2), :] = jnp.concatenate(
                    [e[0:16], shared, f[8:24]], axis=0)
            done = 0 if h0 == 0 else done
            while (done + 1) * 128 <= DH * (h0 + G):
                cs = slice(done * 128, (done + 1) * 128)
                att_ref[t * TQ:(t + 1) * TQ, cs] = ot_ref[t, cs, :].T.astype(BF16)
                done += 1

    def mlp_stages(blk):
        fc = w1_ref.shape[1] // NCH
        b1 = b1_ref[...].astype(F32)[None, :]
        gs, acc = [], []

        def up(c):
            cs = slice(c * fc, (c + 1) * fc)
            gs.append(_gelu(_dot(hn_ref[...], w1_ref[:, cs]) + b1[:, cs]).astype(BF16))

        def down(c):
            if c == 0:
                acc.append(h_ref[...] + b2_ref[...].astype(F32)[None, :])
            acc[0] = acc[0] + _dot(gs[c], w2_ref[c * fc:(c + 1) * fc, :])
            if c == NCH - 1:
                o_ref[rows_of(blk), :] = acc[0].astype(o_ref.dtype)

        return ([functools.partial(up, c) for c in range(NCH)]
                + [functools.partial(down, c) for c in range(NCH)])

    def run(prog, i):
        prog = prog.split()
        stages = mlp_stages(i - 1) if "f" in prog else []
        val, fill = {}, {}

        def do(op):
            if op[0] == "+":
                for name in op[1:].split(","):
                    dma(name).start()
            elif op[0] == "-":
                for name in op[1:].split(","):
                    dma(name).wait()
            elif op == "x":
                x_dma(i + 1).wait()
            elif op == "X":
                for blk in range(3, NS):
                    x_dma(blk).start()
            elif op == "l":
                val["xn"] = ln1(i + 1)
            elif op == "k":
                kb_ref[...] = _bits(_dot(val["xn"], wk_ref[...]).astype(BF16))
            elif op == "p":
                for t in range(NT):
                    replicate_keys(i + 1, t)
            elif op == "q":
                q = _dot(val["xn"], wq_ref[...]) * (DH ** -0.5 * LOG2E)
                qb_ref[...] = _bits(q.T.astype(BF16))
            elif op == "v":
                v = _dot(val["xn"], wv_ref[...])
                for t in range(NT):
                    tile(vt_ref, i + 1, t)[...] = v[t * TQ:(t + 1) * TQ].T
            elif op == "a":
                attention(i, [3] * NT, fill)
            elif op == "a0":
                attention(i, [min(t + 1, 3) for t in range(NT)], fill)
            elif op == "o":
                val["h"] = x_ref[rows_of(i), :].astype(F32) + _dot(att_ref[...], wo_ref[...])
            elif op == "h":
                h_ref[...] = val["h"]
                hn_ref[...] = _layernorm(val["h"]).astype(BF16)
            elif op == "f":
                stages.pop(0)()
            elif op == "s":
                out_dma(i - 1).start()

        for op in prog:
            if "@" in op:
                at, ops = op.split("@")
                fill[int(at)] = lambda ops=ops: [do(o) for o in ops.split("/")]
            else:
                do(op)

    def body(i, carry):
        run(BODY, i)
        return carry

    run(FIRST, -1)
    run(SECOND, 0)
    jax.lax.fori_loop(1, NS - 1, body, 0)
    run(LAST, NS - 1)
    run("f " * (2 * NCH) + "s", NS)
    for blk in range(NS):
        out_dma(blk).wait()


@jax.jit
def pallas_sequential_preLN__sliding_block__dense_activation_gelu__prompt_kernel(
    A_x: jax.Array,
    A_wqkv: jax.Array,
    A_wo: jax.Array,
    B_x: jax.Array,
    B_w1: jax.Array,
    B_b1: jax.Array,
    B_w2: jax.Array,
    B_b2: jax.Array,
):
    del B_x
    B, S, D = A_x.shape
    F = B_w1.shape[1]
    T = TB
    NS, NT = S // T, T // TQ
    assert B == 1 and S % T == 0 and NS >= 3 and D // H == 20
    hbm = pl.BlockSpec(memory_space=pl.ANY)
    out = pl.pallas_call(
        functools.partial(_kernel, T=T, D=D, DH=D // H, NS=NS),
        in_specs=[hbm] * 7,
        out_specs=hbm,
        out_shape=jax.ShapeDtypeStruct((S, D), A_x.dtype),
        scratch_shapes=[
            pltpu.VMEM((S, D), BF16),
            pltpu.VMEM((D, D), BF16),
            pltpu.VMEM((D, D), BF16),
            pltpu.VMEM((D, D), BF16),
            pltpu.VMEM((D, D), BF16),
            pltpu.VMEM((D, F), BF16),
            pltpu.VMEM((F, D), BF16),
            pltpu.VMEM((F,), BF16),
            pltpu.VMEM((D,), BF16),
            pltpu.VMEM((T // 2, D), I32),
            pltpu.VMEM((2, NT, H, TQ // 2, 128), I32),
            pltpu.VMEM((D // 2, T), I32),
            pltpu.VMEM((2, NT, D, TQ), F32),
            pltpu.VMEM((NT, D, TQ), F32),
            pltpu.VMEM((T, D), BF16),
            pltpu.VMEM((T, D), F32),
            pltpu.VMEM((T, D), BF16),
            pltpu.VMEM((S, D), A_x.dtype),
            pltpu.SemaphoreType.DMA((8,)),
            pltpu.SemaphoreType.DMA((NS,)),
            pltpu.SemaphoreType.DMA((NS,)),
        ],
        compiler_params=pltpu.CompilerParams(
            flags={"XLA_TPU_EVENLY_DISTRIBUTE_CRITICAL_NODES": True},
            vmem_limit_bytes=64 * 1024 * 1024,
        ),
    )(A_x.reshape(S, D), A_wqkv, A_wo, B_w1, B_b1, B_w2, B_b2)
    return out.reshape(B, S, D)
```
